```python
import os as _os
_os.environ.setdefault("JAX_PLATFORMS", "cpu")
import jax
import jax.numpy as jnp

def _softmax(x, axis=-1):
    return jax.nn.softmax(x, axis=axis)
def _gelu(x):
    return jax.nn.gelu(x, approximate=True)
def _silu(x):
    return jax.nn.silu(x)
def _sigmoid(x):
    return jax.nn.sigmoid(x)
def _layernorm(x, axis=-1, eps=1e-5):
    m = jnp.mean(x, axis=axis, keepdims=True)
    v = jnp.var(x, axis=axis, keepdims=True)
    return (x - m) / jnp.sqrt(v + eps)
def _scatter_add(tgt, idx, src, axis=0):
    return tgt.at[idx].add(src)
def _segment_sum(src, seg, n):
    return jax.ops.segment_sum(src, seg, n)
class _Rng:
    def __init__(self, key):
        self._k = key
    def _next(self):
        self._k, sub = jax.random.split(self._k)
        return sub
    def normal(self, shape):
        return jax.random.normal(self._next(), shape, dtype=jnp.bfloat16)
    def randint(self, lo, hi, shape):
        return jax.random.randint(self._next(), shape, lo, hi, dtype=jnp.int32)
    def uniform(self, shape, lo=0.0, hi=1.0):
        return jax.random.uniform(self._next(), shape, jnp.bfloat16, lo, hi)
    def permutation(self, n):
        return jax.random.permutation(self._next(), n)


kernel_name = 'parallel_sum__ssm_conv_s5__glu_gated_swiglu__prompt'

def setup_inputs():
    _rng = _Rng(jax.random.key(int.from_bytes(__import__("os").urandom(4), "little")))
    _w = (lambda a: (lambda t: t.astype(jnp.bfloat16) if jnp.issubdtype(t.dtype, jnp.floating) else t)(jnp.asarray(a)))
    def _A_setup():
        B, S, D = 1, 2048, 640
        P = D
        Lambda_re = -0.5 * jnp.exp((lambda *s: _rng.normal(s) * 0.4)(P))
        Lambda_im = (lambda *s: _rng.normal(s) * 0.4)(P) * 1.0
        B_re = (lambda *s: _rng.normal(s) * 0.4)(P, D) * (D ** -0.5)
        B_im = (lambda *s: _rng.normal(s) * 0.4)(P, D) * (D ** -0.5)
        C_re = (lambda *s: _rng.normal(s) * 0.4)(D, P) * (P ** -0.5)
        C_im = (lambda *s: _rng.normal(s) * 0.4)(D, P) * (P ** -0.5)
        log_dt = (lambda *s: _rng.normal(s) * 0.4)(P) * 0.3 - 2.0
        Dskip = (lambda *s: _rng.normal(s) * 0.4)(D)
        return {
            "x": _w((lambda *s: _rng.normal(s) * 0.05)(B, S, D)),
            "Lambda_re": _w(Lambda_re),
            "Lambda_im": _w(Lambda_im),
            "B_re": _w(B_re),
            "B_im": _w(B_im),
            "C_re": _w(C_re),
            "C_im": _w(C_im),
            "log_dt": _w(log_dt),
            "Dskip": _w(Dskip),
        }
    _A_in = _A_setup()

    def _B_setup():
        B, S, D, F = 1, 2048, 640, 1728
        return {
            "x": _w((lambda *s: _rng.normal(s) * 0.05)(B, S, D)),
            "w1": _w((lambda *s: _rng.normal(s) * 0.1)(D, F) * (2.0 / D) ** 0.5),
            "w3": _w((lambda *s: _rng.normal(s) * 0.1)(D, F) * (2.0 / D) ** 0.5),
            "w2": _w((lambda *s: _rng.normal(s) * 0.1)(F, D) * (2.0 / F) ** 0.5),
        }
    _B_in = _B_setup()

    return {
        "A_x": _A_in["x"],
        "A_Lambda_re": _A_in["Lambda_re"],
        "A_Lambda_im": _A_in["Lambda_im"],
        "A_B_re": _A_in["B_re"],
        "A_B_im": _A_in["B_im"],
        "A_C_re": _A_in["C_re"],
        "A_C_im": _A_in["C_im"],
        "A_log_dt": _A_in["log_dt"],
        "A_Dskip": _A_in["Dskip"],
        "B_x": _B_in["x"],
        "B_w1": _B_in["w1"],
        "B_w3": _B_in["w3"],
        "B_w2": _B_in["w2"],
    }

def reference(A_x, A_Lambda_re, A_Lambda_im, A_B_re, A_B_im, A_C_re, A_C_im, A_log_dt, A_Dskip, B_x, B_w1, B_w3, B_w2):
    def _A_ref(x, Lambda_re, Lambda_im, B_re, B_im, C_re, C_im, log_dt, Dskip):
        Bsz, L, H = x.shape
        Lam = Lambda_re + 1j * Lambda_im
        Bmat = B_re + 1j * B_im
        Cmat = C_re + 1j * C_im
        dt = jnp.exp(log_dt)
        Lam_bar = jnp.exp(dt * Lam)
        B_bar = ((Lam_bar - 1.0) / Lam)[:, None] * Bmat
        Bu = jnp.einsum("bld,pd->blp", x + 0j, B_bar)
        h = jnp.zeros_like(Bu[:, 0, :])
        hs = []
        for t in range(L):
            h = Lam_bar[None, :] * h + Bu[:, t, :]
            hs.append(h)
        hseq = jnp.stack(hs, 1)
        y = 2.0 * jnp.einsum("blp,dp->bld", hseq, Cmat).real + x * Dskip[None, None, :]
        return y

    def _B_ref(x, w1, w3, w2):
        gate = jnp.einsum("bsd,df->bsf", x, w1)
        up = jnp.einsum("bsd,df->bsf", x, w3)
        h = _silu(gate) * up
        out = jnp.einsum("bsf,fd->bsd", h, w2)
        return out

    x = A_x
    xn = _layernorm(x, axis=-1)
    return x + _A_ref(xn, A_Lambda_re, A_Lambda_im, A_B_re, A_B_im, A_C_re, A_C_im, A_log_dt, A_Dskip) + _B_ref(xn, B_w1, B_w3, B_w2)
```

```python
import functools
import jax
import jax.numpy as jnp
import jax.experimental.pallas as pl
import jax.experimental.pallas.tpu as pltpu

S, D, P, F = 2048, 640, 640, 1728
NT = D // 128
FM = (F // 128) * 128
FT = F - FM
f32, bf16 = jnp.float32, jnp.bfloat16
_NT_DIMS = (((1,), (1,)), ((), ()))


def _cmul(ar, ai, br, bi):
    return ar * br - ai * bi, ar * bi + ai * br


def _silu_mul(g, u):
    hg = 0.5 * g
    return (hg * jnp.tanh(hg) + hg) * u


def _dot_nt(a, b):
    return jax.lax.dot_general(a, b, _NT_DIMS, preferred_element_type=f32)


def _kernel(x_hbm, lre_hbm, lim_hbm, ldt_hbm, dsk_hbm, bre_hbm, bim_hbm, cre_hbm, cim_hbm,
            w1_hbm, w3_hbm, w2_hbm, o_hbm,
            x_ref, o_ref, lre_ref, lim_ref, ldt_ref, dsk_ref, b_ref, c_ref, w1_ref, w3_ref, wt_ref, w2_ref,
            perm_ref, yperm_ref, xn_ref, bu_ref, h_ref, hh_ref, gu_ref, tmp_ref, sem, *, CH, blocks, FC, SC, OS):
    nb = len(blocks)
    offs = [sum(blocks[:i]) for i in range(nb)]
    TMX = max(blocks)
    nsem = [0]

    def cp(src, dst):
        c = pltpu.make_async_copy(src, dst, sem.at[nsem[0]])
        nsem[0] += 1
        return c

    xc_ = [cp(x_hbm.at[pl.ds(offs[i], blocks[i])], x_ref.at[pl.ds(offs[i], blocks[i])]) for i in range(nb)]
    small = [cp(lre_hbm, lre_ref), cp(lim_hbm, lim_ref), cp(ldt_hbm, ldt_ref), cp(dsk_hbm, dsk_ref)]
    cb = [cp(bre_hbm, b_ref.at[0]), cp(bim_hbm, b_ref.at[1])]
    chunks = list(zip([sum(FC[:i]) for i in range(len(FC))], FC))
    cw = [(cp(w1_hbm.at[pl.ds(s, n)], w1_ref.at[pl.ds(s, n)]), cp(w3_hbm.at[pl.ds(s, n)], w3_ref.at[pl.ds(s, n)]))
          for s, n in chunks]
    cwt = [cp(w1_hbm.at[pl.ds(FM, FT)], wt_ref.at[pl.ds(0, FT)]), cp(w3_hbm.at[pl.ds(FM, FT)], wt_ref.at[pl.ds(FT, FT)])]
    cc = [cp(cre_hbm, c_ref.at[0]), cp(cim_hbm, c_ref.at[1])]
    cw2 = cp(w2_hbm, w2_ref)
    small[3].start()
    xc_[0].start()
    cb[0].start()
    for c in small[:3]:
        c.start()
    cb[1].start()
    oc_ = []

    def layernorm(i):
        TM, o = blocks[i], offs[i]
        L = TM // 8
        dsk = dsk_ref[...].astype(f32).reshape(1, D)
        prev = None
        for k0 in range(0, L, 16):
            for seg in range(8):
                t0 = o + seg * L + k0
                x = x_ref[t0:t0 + 16, :].astype(f32)
                if i > 0 and CH and prev is not None:
                    x = jnp.concatenate([jnp.where(prev < 0.0, prev, x[:, 0:128]), x[:, 128:]], axis=1)
                m = jnp.mean(x, axis=-1, keepdims=True)
                xc = x - m
                v = jnp.mean(xc * xc, axis=-1, keepdims=True)
                rs = jax.lax.rsqrt(v + 1e-5)
                xn = xc * rs
                prev = jnp.broadcast_to(rs, (16, 128))
                o_ref[t0:t0 + 16, :] = x + xn * dsk
                for j in range(NT):
                    for hlf in range(2):
                        perm_ref[j, pl.ds((k0 + hlf * 8) * 8 + seg, 8, stride=8), :] = \
                            xn[hlf * 8:hlf * 8 + 8, j * 128:(j + 1) * 128]
            for j in range(NT):
                xn_ref[i, k0 * 8:k0 * 8 + 128, j * 128:(j + 1) * 128] = perm_ref[j, k0 * 8:k0 * 8 + 128, :].astype(bf16)

    def params():
        lre = lre_ref[...].astype(f32).reshape(1, P)
        lim = lim_ref[...].astype(f32).reshape(1, P)
        dt = jnp.exp(ldt_ref[...].astype(f32).reshape(1, P)).astype(bf16).astype(f32)
        mag = jnp.exp(dt * lre)
        ar = mag * jnp.cos(dt * lim)
        ai = mag * jnp.sin(dt * lim)
        s = jnp.maximum(jnp.abs(lre), jnp.abs(lim))
        lr, li = lre / s, lim / s
        den = (lr * lr + li * li) * s
        nr, ni = ar - 1.0, ai
        cr = (nr * lr + ni * li) / den
        ci = (ni * lr - nr * li) / den
        pw = {}
        pr, pi = ar, ai
        n = 1
        while n < TMX // 8:
            pr, pi = _cmul(pr, pi, pr, pi)
            n *= 2
            pw[n] = (pr, pi)
        return (ar, ai), (cr, ci), pw

    def scan(TM, pw, a, carry):
        L = TM // 8
        row = jax.lax.broadcasted_iota(jnp.int32, (8, P), 0)
        ar, ai = jnp.broadcast_to(a[0], (8, P)), jnp.broadcast_to(a[1], (8, P))
        ers, eis = [], []
        for j in range(NT):
            cs = slice(j * 128, (j + 1) * 128)
            er, ei = bu_ref[0, 0:8, cs], bu_ref[1, 0:8, cs]
            if ers:
                er = jnp.where(jnp.abs(ers[-1]) < 0.0, ers[-1], er)
            for k in range(1, L):
                br, bi = bu_ref[0, k * 8:k * 8 + 8, cs], bu_ref[1, k * 8:k * 8 + 8, cs]
                er, ei = (ar[:, cs] * er + br) - ai[:, cs] * ei, (ar[:, cs] * ei + bi) + ai[:, cs] * er
            ers.append(er); eis.append(ei)
        er, ei = jnp.concatenate(ers, axis=1), jnp.concatenate(eis, axis=1)
        qr, qi = (jnp.broadcast_to(t, (8, P)) for t in pw[L])
        if carry is None:
            cr_ = ci_ = jnp.zeros((8, P), f32)
        else:
            cr_, ci_ = carry
            tr, ti = _cmul(qr, qi, cr_, ci_)
            er = er + jnp.where(row == 0, tr, 0.0)
            ei = ei + jnp.where(row == 0, ti, 0.0)
        sh = 1
        while sh < 8:
            rr = jnp.where(row >= sh, pltpu.roll(er, sh, 0), 0.0)
            ri = jnp.where(row >= sh, pltpu.roll(ei, sh, 0), 0.0)
            tr, ti = _cmul(qr, qi, rr, ri)
            er, ei = er + tr, ei + ti
            qr, qi = _cmul(qr, qi, qr, qi)
            sh *= 2
        hr = jnp.where(row == 0, cr_, pltpu.roll(er, 1, 0))
        hi = jnp.where(row == 0, ci_, pltpu.roll(ei, 1, 0))
        carry = (jnp.broadcast_to(er[7:8, :], (8, P)), jnp.broadcast_to(ei[7:8, :], (8, P)))
        for k in range(L):
            br, bi = bu_ref[0, k * 8:k * 8 + 8, :], bu_ref[1, k * 8:k * 8 + 8, :]
            hr, hi = (ar * hr + br) - ai * hi, (ar * hi + bi) + ai * hr
            if k % 2 == 0:
                pr_, pi_ = hr, hi
            else:
                h_ref[0, (k - 1) * 8:(k + 1) * 8, :] = jnp.concatenate([pr_, hr], axis=0).astype(bf16)
                h_ref[1, (k - 1) * 8:(k + 1) * 8, :] = jnp.concatenate([pi_, hi], axis=0).astype(bf16)
        return carry

    xc_[0].wait()
    small[3].wait()
    cb[0].wait()
    for a, b in cw[:2]:
        a.start(); b.start()
    layernorm(0)
    carry = None
    for i in range(nb):
        TM, o = blocks[i], offs[i]
        L = TM // 8
        xp = xn_ref[i, 0:TM, :]
        bu_ref[0, 0:TM] = _dot_nt(xp, b_ref[0])
        if i == 0:
            cb[1].wait()
            for c in small[:3]:
                c.wait()
            for a, b in cw[2:]:
                a.start(); b.start()
            for c in cwt + cc + [cw2] + xc_[1:2]:
                c.start()
        bu_ref[1, 0:TM] = _dot_nt(xp, b_ref[1])
        if i > 0:
            c = cp(o_ref.at[pl.ds(offs[i - 1], blocks[i - 1])], o_hbm.at[pl.ds(offs[i - 1], blocks[i - 1])])
            c.start(); oc_.append(c)
            if i + 1 < nb:
                xc_[i + 1].wait()
        pend = None
        for ci_idx, (s, n) in enumerate(chunks):
            if i == 0:
                cw[ci_idx][0].wait(); cw[ci_idx][1].wait()
                if ci_idx == len(chunks) - 1:
                    for c in cwt + cc + [cw2, xc_[1]]:
                        c.wait()
                    for c in xc_[2:]:
                        c.start()
            if ci_idx == SC:
                if i == 0:
                    a, (c_r, c_i), pw = params()
                carry = scan(TM, pw, a, carry)
            g = _dot_nt(xp, w1_ref[s:s + n, :])
            u = _dot_nt(xp, w3_ref[s:s + n, :])
            if i == 0:
                if pend is not None:
                    ps, pn = pend
                    g_, u_ = gu_ref[0, :, ps:ps + pn], gu_ref[1, :, ps:ps + pn]
                    hh_ref[0:TM, ps:ps + pn] = _silu_mul(g_, u_).astype(bf16)
                    pend = None
            if i == 0 and ci_idx < len(chunks) - 1:
                gu_ref[0, :, s:s + n] = g
                gu_ref[1, :, s:s + n] = u
                pend = (s, n)
            else:
                hh_ref[0:TM, s:s + n] = _silu_mul(g, u).astype(bf16)
        gu = _dot_nt(xp, wt_ref[...])
        u = pltpu.roll(gu, FT, 1)
        hh_ref[0:TM, FM:F] = _silu_mul(gu, u)[:, 0:FT].astype(bf16)
        if i == 0:
            p_r, p_i = _cmul(c_ref[0].astype(f32), c_ref[1].astype(f32), 2.0 * c_r, 2.0 * c_i)
            c_ref[0] = p_r.astype(bf16)
            c_ref[1] = (-p_i).astype(bf16)
        if i + 1 < nb:
            layernorm(i + 1)
        for j in range(NT):
            cs = slice(j * 128, (j + 1) * 128)
            y = jnp.dot(hh_ref[0:TM, :], w2_ref[:, cs], preferred_element_type=f32)
            y = y + _dot_nt(h_ref[0, 0:TM], c_ref[0, cs, :])
            y = y + _dot_nt(h_ref[1, 0:TM], c_ref[1, cs, :])
            yperm_ref[j, 0:TM] = y
            for r in range(TM // 8):
                t0 = r * 8
                seg, k0 = t0 // L, t0 % L
                o_ref[o + t0:o + t0 + 8, cs] += yperm_ref[j, pl.ds(k0 * 8 + seg, 8, stride=8), :]
            if i == nb - 1 and j in OS:
                j0 = ([0] + [t + 1 for t in OS])[OS.index(j)]
                cs = slice(j0 * 128, (j + 1) * 128)
                c = cp(o_ref.at[pl.ds(o, TM), cs], o_hbm.at[pl.ds(o, TM), cs])
                c.start(); oc_.append(c)
    for c in oc_:
        c.wait()


def _build(cfg=2, fc=0, SC=2, os=1, CH=1):
    FC = [[512, 640, 512], [256, 512, 512, 384], [640, 640, 384], [512,512,384,256]][fc]
    OS = [[4], [3, 4], [1,3,4]][os]
    blocks = [[512] * 4, [256] * 8, [512, 512, 512, 256, 256], [1024, 1024], [512,512,512,256,128,128]][cfg]
    TMX = max(blocks)
    nb = len(blocks)

    def fn(A_x, A_Lambda_re, A_Lambda_im, A_B_re, A_B_im, A_C_re, A_C_im, A_log_dt, A_Dskip, B_x, B_w1, B_w3, B_w2):
        hbm = pl.BlockSpec(memory_space=pltpu.HBM)
        V = pltpu.VMEM
        out = pl.pallas_call(
            functools.partial(_kernel, CH=CH, blocks=blocks, FC=FC, SC=SC, OS=OS),
            in_specs=[hbm] * 12,
            out_specs=hbm,
            out_shape=jax.ShapeDtypeStruct((S, D), f32),
            scratch_shapes=[V((S, D), bf16), V((S, D), f32), V((P,), bf16), V((P,), bf16), V((P,), bf16), V((D,), bf16),
                            V((2, P, D), bf16), V((2, D, P), bf16), V((FM, D), bf16), V((FM, D), bf16), V((128, D), bf16),
                            V((F, D), bf16),
                            V((NT, TMX, 128), f32), V((NT, TMX, 128), f32), V((nb, TMX, D), bf16),
                            V((2, TMX, P), f32), V((2, TMX, P), bf16), V((TMX, F), bf16), V((2, blocks[0], FM), f32), V((16, 128), f32),
                            pltpu.SemaphoreType.DMA((64,))],
            compiler_params=pltpu.CompilerParams(vmem_limit_bytes=100 * 1024 * 1024),
        )(A_x.reshape(S, D), A_Lambda_re, A_Lambda_im, A_log_dt, A_Dskip, A_B_re, A_B_im, A_C_re, A_C_im,
          B_w1.T, B_w3.T, B_w2)
        return out.reshape(1, S, D)
    return fn


@jax.jit
def pallas_parallel_sum__ssm_conv_s5__glu_gated_swiglu__prompt_kernel(
        A_x, A_Lambda_re, A_Lambda_im, A_B_re, A_B_im, A_C_re, A_C_im, A_log_dt, A_Dskip, B_x, B_w1, B_w3, B_w2):
    return _build()(A_x, A_Lambda_re, A_Lambda_im, A_B_re, A_B_im, A_C_re, A_C_im, A_log_dt, A_Dskip,
                    B_x, B_w1, B_w3, B_w2)
```
